```python
import os as _os
_os.environ.setdefault("JAX_PLATFORMS", "cpu")
import jax
import jax.numpy as jnp

def _softmax(x, axis=-1):
    return jax.nn.softmax(x, axis=axis)
def _gelu(x):
    return jax.nn.gelu(x, approximate=True)
def _silu(x):
    return jax.nn.silu(x)
def _sigmoid(x):
    return jax.nn.sigmoid(x)
def _layernorm(x, axis=-1, eps=1e-5):
    m = jnp.mean(x, axis=axis, keepdims=True)
    v = jnp.var(x, axis=axis, keepdims=True)
    return (x - m) / jnp.sqrt(v + eps)
def _scatter_add(tgt, idx, src, axis=0):
    return tgt.at[idx].add(src)
def _segment_sum(src, seg, n):
    return jax.ops.segment_sum(src, seg, n)
class _Rng:
    def __init__(self, key):
        self._k = key
    def _next(self):
        self._k, sub = jax.random.split(self._k)
        return sub
    def normal(self, shape):
        return jax.random.normal(self._next(), shape, dtype=jnp.bfloat16)
    def randint(self, lo, hi, shape):
        return jax.random.randint(self._next(), shape, lo, hi, dtype=jnp.int32)
    def uniform(self, shape, lo=0.0, hi=1.0):
        return jax.random.uniform(self._next(), shape, jnp.bfloat16, lo, hi)
    def permutation(self, n):
        return jax.random.permutation(self._next(), n)


kernel_name = 'standalone__mha_softmax__near_ridge'

def setup_inputs():
    _rng = _Rng(jax.random.key(int.from_bytes(__import__("os").urandom(4), "little")))
    _w = (lambda a: (lambda t: t.astype(jnp.bfloat16) if jnp.issubdtype(t.dtype, jnp.floating) else t)(jnp.asarray(a)))
    B, H, Sq, Sk, D = 32, 32, 288, 512, 128
    return {
        "q": _w((lambda *s: _rng.normal(s) * 0.4)(B, H, Sq, D)),
        "k": _w((lambda *s: _rng.normal(s) * 0.4)(B, H, Sk, D)),
        "v": _w((lambda *s: _rng.normal(s) * 0.05)(B, H, Sk, D)),
    }

def reference(q, k, v):
    scale = q.shape[-1] ** -0.5
    scores = jnp.einsum("bhqd,bhkd->bhqk", q, k) * scale
    p = _softmax(scores, axis=-1)
    return jnp.einsum("bhqk,bhkd->bhqd", p, v)
```

```python
import math

import jax
import jax.numpy as jnp
from jax import lax
import jax.experimental.pallas as pl
import jax.experimental.pallas.tpu as pltpu

HB = 8
RING = 8
NS = 8
CR = 144


def _attend(q_ref, k_ref, v_ref, o_ref):
    hb, sq, d = q_ref.shape
    c = (d ** -0.5) * math.log2(math.e)
    for h in range(hb):
        q = q_ref[h]
        k = k_ref[h]
        v = v_ref[h]
        s = lax.dot_general(q, k, (((1,), (1,)), ((), ())),
                            preferred_element_type=jnp.float32)
        m = jnp.max(s, axis=-1, keepdims=True)
        p = jnp.exp2((s - m) * c)
        l = jnp.sum(p, axis=-1, keepdims=True)
        o = jnp.dot(p.astype(jnp.bfloat16), v, preferred_element_type=jnp.float32)
        o_ref[pl.ds(h * sq, sq), :] = (o * pl.reciprocal(l, approx=False)).astype(o_ref.dtype)


def _kernel(q_hbm, k_hbm, v_hbm, o_hbm, qb, kb, vb, ob, sem_in, sem_out):
    n = q_hbm.shape[0]
    groups = o_hbm.shape[0]
    per_group = o_hbm.shape[2] // CR

    def in_copies(i, slot):
        return [pltpu.make_async_copy(src.at[i], dst.at[slot], sem_in.at[slot, j])
                for j, (src, dst) in enumerate(((q_hbm, qb), (k_hbm, kb), (v_hbm, vb)))]

    def start_write(w, carry):
        g = w // per_group
        rows = pl.ds(pl.multiple_of((w % per_group) * CR, 16), CR)
        pltpu.make_async_copy(ob.at[g, :, rows, :], o_hbm.at[g, :, rows, :],
                              sem_out.at[g]).start()
        return carry

    for j in range(RING):
        for cp in in_copies(j, j):
            cp.start()

    j0 = n - RING
    ready = (j0 // NS) * per_group
    per_step = -(-ready // RING)

    def body(i, carry):
        slot = i % RING

        @pl.when(i < j0)
        def _():
            for cp in in_copies(i, slot):
                cp.wait()

        @pl.when(i == j0)
        def _():
            for j in range(j0, n):
                for cp in in_copies(j, j % RING):
                    cp.wait()

        @pl.when(i >= j0)
        def _():
            lo = (i - j0) * per_step
            lax.fori_loop(lo, jnp.minimum(lo + per_step, ready), start_write, 0)

        _attend(qb.at[slot], kb.at[slot], vb.at[slot], ob.at[i // NS, i % NS])

        @pl.when(i + RING < n)
        def _():
            for cp in in_copies(i + RING, slot):
                cp.start()

        return carry

    lax.fori_loop(0, n, body, 0)
    lax.fori_loop(ready, groups * per_group, start_write, 0)
    for g in range(groups):
        pltpu.make_async_copy(ob.at[g], o_hbm.at[g], sem_out.at[g]).wait()


@jax.jit
def pallas_standalone__mha_softmax__near_ridge_kernel(
    q: jax.Array,
    k: jax.Array,
    v: jax.Array,
):
    b, h, sq, d = q.shape
    sk = k.shape[2]
    n = b * h // HB
    groups = n // NS
    out = pl.pallas_call(
        _kernel,
        in_specs=[pl.BlockSpec(memory_space=pl.ANY)] * 3,
        out_specs=pl.BlockSpec(memory_space=pl.ANY),
        out_shape=jax.ShapeDtypeStruct((groups, NS, HB * sq, d), q.dtype),
        scratch_shapes=[
            pltpu.VMEM((RING, HB, sq, d), q.dtype),
            pltpu.VMEM((RING, HB, sk, d), k.dtype),
            pltpu.VMEM((RING, HB, sk, d), v.dtype),
            pltpu.VMEM((groups, NS, HB * sq, d), q.dtype),
            pltpu.SemaphoreType.DMA((RING, 3)),
            pltpu.SemaphoreType.DMA((groups,)),
        ],
        compiler_params=pltpu.CompilerParams(vmem_limit_bytes=120 * 1024 * 1024),
    )(q.reshape(n, HB, sq, d), k.reshape(n, HB, sk, d), v.reshape(n, HB, sk, d))
    return out.reshape(b, h, sq, d)
```

```python
import math

import jax
import jax.numpy as jnp
from jax import lax
import jax.experimental.pallas as pl
import jax.experimental.pallas.tpu as pltpu

HB = 8
LOOKAHEAD = 150
PERIOD = ((1, 128, 0), (2, 128, 1), (1, 128, 0), (2, 128, 1), (0, 144, 1))
W_STREAMS = 8
W_STRIDE = 4096
W_ROWS = 128
W_FIRST = 48
W_STEP = 16


def _read_schedule(sq, sk):
    rows = (HB * sq, HB * sk, HB * sk)
    off = [0, 0, 0]
    descs = []
    while off[0] < rows[0]:
        for a, r, t in PERIOD:
            descs.append((a, off[a], r, t))
            off[a] += r
    assert tuple(off) == rows
    return descs


def _make_kernel(sq, sk, d):
    descs = _read_schedule(sq, sk)
    nd = len(descs)
    ahead, extra = divmod(LOOKAHEAD, nd)
    assert extra > 0
    ring = ahead + 2
    scale = (d ** -0.5) * math.log2(math.e)

    def kernel(q_hbm, k_hbm, v_hbm, o_hbm, qb, kb, vb, ob, sem_in, sem_out):
        n = q_hbm.shape[0]
        groups = o_hbm.shape[0]
        per_group = W_STRIDE // W_ROWS
        hbm = (q_hbm, k_hbm, v_hbm)
        bufs = (qb, kb, vb)
        ob_rows = ob.reshape(groups * W_STREAMS * W_STRIDE, d)

        def start_reads(lo, hi, i, slots):
            for t in range(lo, hi):
                dc, di = divmod(t, nd)
                a, off, r, thread = descs[di]
                pltpu.make_async_copy(
                    hbm[a].at[i + dc, pl.ds(off, r), :],
                    bufs[a].at[slots[dc], pl.ds(off, r), :],
                    sem_in.at[slots[dc], a],
                ).start(priority=thread)

        def wait_reads(slot):
            for a in range(3):
                pltpu.make_async_copy(
                    bufs[a].at[slot], bufs[a].at[slot], sem_in.at[slot, a]).wait()

        def start_write(w, carry):
            g = w // per_group
            rows = pl.ds(pl.multiple_of((w % per_group) * W_ROWS, 16), W_ROWS)
            pltpu.make_async_copy(
                ob.at[g, :, rows, :], o_hbm.at[g, :, rows, :], sem_out.at[g]).start()
            return carry

        def attend(i, slot, after_head):
            base = i * (HB * sq)
            for h in range(HB):
                q = qb[slot, pl.ds(h * sq, sq), :]
                k = kb[slot, pl.ds(h * sk, sk), :]
                v = vb[slot, pl.ds(h * sk, sk), :]
                s = lax.dot_general(q, k, (((1,), (1,)), ((), ())),
                                    preferred_element_type=jnp.float32)
                m = jnp.max(s, axis=-1, keepdims=True)
                p = jnp.exp2((s - m) * scale)
                l = jnp.sum(p, axis=-1, keepdims=True)
                o = jnp.dot(p.astype(v.dtype), v, preferred_element_type=jnp.float32)
                o = o * pl.reciprocal(l, approx=True)
                ob_rows[pl.ds(pl.multiple_of(base + h * sq, 16), sq), :] = o.astype(ob.dtype)
                after_head(h)

        start_reads(0, LOOKAHEAD, 0, list(range(ring)))
        n_main = n - ahead - 1

        def main_step(i, carry):
            slots = {dc: (i + dc) % ring for dc in (ahead, ahead + 1)}
            wait_reads(i % ring)
            attend(i, i % ring, lambda h: start_reads(
                LOOKAHEAD + (h * nd) // HB, LOOKAHEAD + ((h + 1) * nd) // HB, i, slots))
            return carry

        lax.fori_loop(0, n_main, main_step, 0)
        start_reads(extra, nd, n - 1, {0: (n - 1) % ring})

        for j in range(n_main, n):
            wait_reads(j % ring)
        done_groups = (n_main * HB * sq) // (W_STREAMS * W_STRIDE)
        early = W_FIRST + (n - n_main) * W_STEP
        assert early <= done_groups * per_group
        lax.fori_loop(0, W_FIRST, start_write, 0)

        def tail_step(i, carry):
            attend(i, i % ring, lambda h: None)
            lo = W_FIRST + (i - n_main) * W_STEP
            lax.fori_loop(lo, lo + W_STEP, start_write, 0)
            return carry

        lax.fori_loop(n_main, n, tail_step, 0)
        lax.fori_loop(early, groups * per_group, start_write, 0)
        for g in range(groups):
            pltpu.make_async_copy(ob.at[g], o_hbm.at[g], sem_out.at[g]).wait()

    return kernel, ring


@jax.jit
def pallas_standalone__mha_softmax__near_ridge_kernel(
    q: jax.Array,
    k: jax.Array,
    v: jax.Array,
):
    b, h, sq, d = q.shape
    sk = k.shape[2]
    n = b * h // HB
    groups = b * h * sq // (W_STREAMS * W_STRIDE)
    kernel, ring = _make_kernel(sq, sk, d)
    out = pl.pallas_call(
        kernel,
        in_specs=[pl.BlockSpec(memory_space=pl.ANY)] * 3,
        out_specs=pl.BlockSpec(memory_space=pl.ANY),
        out_shape=jax.ShapeDtypeStruct((groups, W_STREAMS, W_STRIDE, d), q.dtype),
        scratch_shapes=[
            pltpu.VMEM((ring, HB * sq, d), q.dtype),
            pltpu.VMEM((ring, HB * sk, d), k.dtype),
            pltpu.VMEM((ring, HB * sk, d), v.dtype),
            pltpu.VMEM((groups, W_STREAMS, W_STRIDE, d), q.dtype),
            pltpu.SemaphoreType.DMA((ring, 3)),
            pltpu.SemaphoreType.DMA((groups,)),
        ],
        compiler_params=pltpu.CompilerParams(
            vmem_limit_bytes=100 * 1024 * 1024,
            disable_bounds_checks=True,
        ),
    )(q.reshape(n, HB * sq, d), k.reshape(n, HB * sk, d), v.reshape(n, HB * sk, d))
    return out.reshape(b, h, sq, d)
```

```python
import math

import jax
import jax.numpy as jnp
from jax import lax
import jax.experimental.pallas as pl
import jax.experimental.pallas.tpu as pltpu

HB = 8
LOOKAHEAD = 154
BLK = 256
SHIFT = 112
W_STREAMS = 8
W_STRIDE = 4096
W_ROWS = 128
W_FIRST = 48
W_STEP = 16


def _read_schedule(sq, sk):
    nblk = HB * sk // BLK
    q_rows = HB * sq // nblk
    assert nblk * BLK == HB * sk and q_rows * nblk == HB * sq and q_rows % 16 == 0
    descs = []
    for j in range(nblk):
        lo = (0, j * BLK + SHIFT, BLK - SHIFT)
        hi = (0, (j + 1) * BLK, SHIFT) if j + 1 < nblk else (1, 0, SHIFT)
        descs += [(1,) + lo, (2,) + lo, (1,) + hi, (2,) + hi, (0, 0, j * q_rows, q_rows)]
    return [desc + (t % 2,) for t, desc in enumerate(descs)]


def _make_kernel(sq, sk, d):
    descs = _read_schedule(sq, sk)
    nd = len(descs)
    ahead, extra = divmod(LOOKAHEAD, nd)
    assert 0 < extra <= nd - 5
    ring = ahead + 2
    scale = (d ** -0.5) * math.log2(math.e)

    def kernel(q_hbm, k_hbm, v_hbm, o_hbm, qb, kb, vb, ob, sem_in, sem_out):
        n = q_hbm.shape[0]
        groups = o_hbm.shape[0]
        per_group = W_STRIDE // W_ROWS
        hbm = (q_hbm, k_hbm, v_hbm)
        bufs = (qb, kb, vb)
        ob_rows = ob.reshape(groups * W_STREAMS * W_STRIDE, d)

        def start_read(a, chunk, slot, row, rows, thread):
            pltpu.make_async_copy(
                hbm[a].at[chunk, pl.ds(row, rows), :],
                bufs[a].at[slot, pl.ds(row, rows), :],
                sem_in.at[slot, a],
            ).start(priority=thread)

        def start_reads(lo, hi, i, slots):
            for t in range(lo, hi):
                dc, di = divmod(t, nd)
                a, spill, row, rows, thread = descs[di]
                if dc + spill in slots:
                    start_read(a, i + dc + spill, slots[dc + spill], row, rows, thread)

        def wait_reads(slot):
            for a in range(3):
                pltpu.make_async_copy(
                    bufs[a].at[slot], bufs[a].at[slot], sem_in.at[slot, a]).wait()

        def start_write(w, carry):
            g = w // per_group
            rows = pl.ds(pl.multiple_of((w % per_group) * W_ROWS, 16), W_ROWS)
            pltpu.make_async_copy(
                ob.at[g, :, rows, :], o_hbm.at[g, :, rows, :], sem_out.at[g]).start()
            return carry

        def attend(i, slot, after_head):
            base = i * (HB * sq)
            for h in range(HB):
                q = qb[slot, pl.ds(h * sq, sq), :]
                k = kb[slot, pl.ds(h * sk, sk), :]
                v = vb[slot, pl.ds(h * sk, sk), :]
                s = lax.dot_general(q, k, (((1,), (1,)), ((), ())),
                                    preferred_element_type=jnp.float32)
                m = jnp.max(s, axis=-1, keepdims=True)
                p = jnp.exp2((s - m) * scale)
                l = jnp.sum(p, axis=-1, keepdims=True)
                o = jnp.dot(p.astype(v.dtype), v, preferred_element_type=jnp.float32)
                r = pl.reciprocal(l, approx=True)
                r = r * (2.0 - l * r)
                ob_rows[pl.ds(pl.multiple_of(base + h * sq, 16), sq), :] = (
                    (o * r).astype(ob.dtype))
                after_head(h)

        start_read(1, 0, 0, 0, SHIFT, 0)
        start_read(2, 0, 0, 0, SHIFT, 1)
        start_reads(0, LOOKAHEAD, 0, {c: c for c in range(ring)})
        n_main = n - ahead - 1

        def main_step(i, carry):
            slots = {dc: (i + dc) % ring for dc in (ahead, ahead + 1)}
            wait_reads(i % ring)
            attend(i, i % ring, lambda h: start_reads(
                LOOKAHEAD + (h * nd) // HB, LOOKAHEAD + ((h + 1) * nd) // HB, i, slots))
            return carry

        lax.fori_loop(0, n_main, main_step, 0)
        start_reads(extra, nd, n - 1, {0: (n - 1) % ring})

        for j in range(n_main, n):
            wait_reads(j % ring)
        done_groups = (n_main * HB * sq) // (W_STREAMS * W_STRIDE)
        early = W_FIRST + (n - n_main) * W_STEP
        assert early <= done_groups * per_group
        lax.fori_loop(0, W_FIRST, start_write, 0)

        def tail_step(i, carry):
            attend(i, i % ring, lambda h: None)
            lo = W_FIRST + (i - n_main) * W_STEP
            lax.fori_loop(lo, lo + W_STEP, start_write, 0)
            return carry

        lax.fori_loop(n_main, n, tail_step, 0)
        lax.fori_loop(early, groups * per_group, start_write, 0)
        for g in range(groups):
            pltpu.make_async_copy(ob.at[g], o_hbm.at[g], sem_out.at[g]).wait()

    return kernel, ring


@jax.jit
def pallas_standalone__mha_softmax__near_ridge_kernel(
    q: jax.Array,
    k: jax.Array,
    v: jax.Array,
):
    b, h, sq, d = q.shape
    sk = k.shape[2]
    n = b * h // HB
    groups = b * h * sq // (W_STREAMS * W_STRIDE)
    kernel, ring = _make_kernel(sq, sk, d)
    out = pl.pallas_call(
        kernel,
        in_specs=[pl.BlockSpec(memory_space=pl.ANY)] * 3,
        out_specs=pl.BlockSpec(memory_space=pl.ANY),
        out_shape=jax.ShapeDtypeStruct((groups, W_STREAMS, W_STRIDE, d), q.dtype),
        scratch_shapes=[
            pltpu.VMEM((ring, HB * sq, d), q.dtype),
            pltpu.VMEM((ring, HB * sk, d), k.dtype),
            pltpu.VMEM((ring, HB * sk, d), v.dtype),
            pltpu.VMEM((groups, W_STREAMS, W_STRIDE, d), q.dtype),
            pltpu.SemaphoreType.DMA((ring, 3)),
            pltpu.SemaphoreType.DMA((groups,)),
        ],
        compiler_params=pltpu.CompilerParams(
            vmem_limit_bytes=100 * 1024 * 1024,
            disable_bounds_checks=True,
        ),
    )(q.reshape(n, HB * sq, d), k.reshape(n, HB * sk, d), v.reshape(n, HB * sk, d))
    return out.reshape(b, h, sq, d)
```

```python
import math

import jax
import jax.numpy as jnp
from jax import lax
import jax.experimental.pallas as pl
import jax.experimental.pallas.tpu as pltpu

HB = 16
LANES = 4
DEPTH = 70
BLK = 256
QBLK = 128
SHIFT = 104
W_STREAMS = 8
W_STRIDE = 4096
W_ROWS = 128
W_FIRST = 48
W_STEP = 16


def _lane_visits(lane, rows):
    def cut(a, start, count):
        if start >= rows[a]:
            return [(a, lane, 1, start - rows[a], count)]
        if start + count <= rows[a]:
            return [(a, lane, 0, start, count)]
        return [(a, lane, 0, start, rows[a] - start),
                (a, lane, 1, 0, start + count - rows[a])]

    def block(a, j):
        return cut(a, j * BLK + SHIFT, BLK - SHIFT) + cut(a, (j + 1) * BLK, SHIFT)

    nblk, nq = rows[1] // BLK, rows[0] // QBLK
    assert nblk * BLK == rows[1] == rows[2] and nq * QBLK == rows[0]
    qs = [cut(0, j * QBLK + SHIFT % QBLK, QBLK) for j in range(nq)]
    rounds = []
    for j in range(nblk):
        mine = qs[j * nq // nblk:(j + 1) * nq // nblk]
        if lane % 2 == 0:
            rounds.append([block(1, j)] + mine[:-1] + [block(2, j)] + mine[-1:])
        else:
            rounds.append(mine[:1] + [block(1, j)] + mine[1:] + [block(2, j)])
    return rounds


def _read_schedule(rows):
    lanes = [_lane_visits(lane, rows) for lane in range(LANES)]
    threads = []
    for t in range(2):
        threads.append([copy + (t,)
                        for rounds in zip(*lanes[t::2])
                        for visits in rounds
                        for visit in visits
                        for copy in visit])
    assert len(threads[0]) == len(threads[1])
    return [copy for pair in zip(*threads) for copy in pair]


def _make_kernel(sq, sk, d):
    hl = HB // LANES
    rows = (hl * sq, hl * sk, hl * sk)
    base = (0, rows[0], rows[0] + rows[1])
    sched = _read_schedule(rows)
    nd = len(sched)
    assert all(not spill for _, _, spill, _, _, _ in sched[:DEPTH])
    ring = 3
    scale = (d ** -0.5) * math.log2(math.e)

    def kernel(q_hbm, k_hbm, v_hbm, o_hbm, buf, ob, sem_in, sem_out):
        n = q_hbm.shape[1]
        groups = o_hbm.shape[0]
        group_rows = W_STREAMS * W_STRIDE
        per_group = W_STRIDE // W_ROWS
        lane_rows = n * rows[0]
        hbm = (q_hbm, k_hbm, v_hbm)
        ob_rows = ob.reshape(groups * group_rows, d)

        def start_read(copy, chunk, slot):
            a, lane, _, row, count, thread = copy
            pltpu.make_async_copy(
                hbm[a].at[lane, chunk, pl.ds(row, count), :],
                buf.at[slot, lane, pl.ds(base[a] + row, count), :],
                sem_in.at[slot],
            ).start(priority=thread)

        def start_reads(lo, hi, i, slots):
            for t in range(lo, hi):
                copy = sched[t % nd]
                ahead = t // nd + copy[2]
                if ahead in slots:
                    start_read(copy, i + ahead, slots[ahead])

        def wait_reads(slot):
            pltpu.make_async_copy(buf.at[slot], buf.at[slot], sem_in.at[slot]).wait()

        def attend(i, slot, after_head):
            for h in range(HB):
                lane, hh = divmod(h, hl)
                q = buf[slot, lane, pl.ds(base[0] + hh * sq, sq), :]
                k = buf[slot, lane, pl.ds(base[1] + hh * sk, sk), :]
                v = buf[slot, lane, pl.ds(base[2] + hh * sk, sk), :]
                s = lax.dot_general(q, k, (((1,), (1,)), ((), ())),
                                    preferred_element_type=jnp.float32)
                m = jnp.max(s, axis=-1, keepdims=True)
                p = jnp.exp2((s - m) * scale)
                l = jnp.sum(p, axis=-1, keepdims=True)
                o = jnp.dot(p.astype(v.dtype), v, preferred_element_type=jnp.float32)
                r = pl.reciprocal(l, approx=True)
                r = r * (2.0 - l * r)
                row = lane * lane_rows + (i * hl + hh) * sq
                ob_rows[pl.ds(pl.multiple_of(row, 16), sq), :] = (o * r).astype(ob.dtype)
                after_head(h)

        n_main = n - 2
        pending = [(s * lane_rows + n_main * rows[0], (s + 1) * lane_rows)
                   for s in range(LANES)]
        done = [g for g in range(groups)
                if not any(g * group_rows < hi and lo < (g + 1) * group_rows
                           for lo, hi in pending)]
        order = done + [g for g in range(groups) if g not in done]
        early = W_FIRST + (n - n_main) * W_STEP
        assert early <= len(done) * per_group

        def start_write(w, carry):
            j = w // per_group
            g = jnp.int32(order[0])
            for u in range(1, groups):
                g = jnp.where(j >= u, order[u], g)
            part = pl.ds(pl.multiple_of((w % per_group) * W_ROWS, 16), W_ROWS)
            pltpu.make_async_copy(
                ob.at[g, :, part, :], o_hbm.at[g, :, part, :], sem_out).start()
            return carry

        lead = nd + DEPTH
        for copy in sched:
            if copy[2]:
                start_read(copy, 0, 0)
        start_reads(0, lead, 0, {0: 0, 1: 1})

        def main_step(i, carry):
            slots = {ahead: (i + ahead) % ring for ahead in (1, 2)}
            wait_reads(i % ring)
            attend(i, i % ring, lambda h: start_reads(
                lead + (h * nd) // HB, lead + ((h + 1) * nd) // HB, i, slots))
            return carry

        lax.fori_loop(0, n_main, main_step, 0)
        start_reads(DEPTH, nd, n - 1, {0: (n - 1) % ring})
        lax.fori_loop(0, W_FIRST, start_write, 0)
        for j in range(n_main, n):
            wait_reads(j % ring)

        def tail_step(i, carry):
            attend(i, i % ring, lambda h: None)
            lo = W_FIRST + (i - n_main) * W_STEP
            lax.fori_loop(lo, lo + W_STEP, start_write, 0)
            return carry

        lax.fori_loop(n_main, n, tail_step, 0)
        lax.fori_loop(early, groups * per_group, start_write, 0)
        pltpu.make_async_copy(ob, o_hbm, sem_out).wait()

    return kernel, ring, rows


@jax.jit
def pallas_standalone__mha_softmax__near_ridge_kernel(
    q: jax.Array,
    k: jax.Array,
    v: jax.Array,
):
    b, h, sq, d = q.shape
    sk = k.shape[2]
    n = b * h // HB
    groups = b * h * sq // (W_STREAMS * W_STRIDE)
    kernel, ring, rows = _make_kernel(sq, sk, d)
    out = pl.pallas_call(
        kernel,
        in_specs=[pl.BlockSpec(memory_space=pl.ANY)] * 3,
        out_specs=pl.BlockSpec(memory_space=pl.ANY),
        out_shape=jax.ShapeDtypeStruct((groups, W_STREAMS, W_STRIDE, d), q.dtype),
        scratch_shapes=[
            pltpu.VMEM((ring, LANES, sum(rows), d), q.dtype),
            pltpu.VMEM((groups, W_STREAMS, W_STRIDE, d), q.dtype),
            pltpu.SemaphoreType.DMA((ring,)),
            pltpu.SemaphoreType.DMA(()),
        ],
        compiler_params=pltpu.CompilerParams(
            vmem_limit_bytes=104 * 1024 * 1024,
            disable_bounds_checks=True,
        ),
    )(q.reshape(LANES, n, rows[0], d),
      k.reshape(LANES, n, rows[1], d),
      v.reshape(LANES, n, rows[2], d))
    return out.reshape(b, h, sq, d)
```

```python
import math

import jax
import jax.numpy as jnp
from jax import lax
import jax.experimental.pallas as pl
import jax.experimental.pallas.tpu as pltpu

HB = 16
LANES = 4
RING = 3
DEPTH = 70
BLK = 256
QBLK = 128
SHIFT = 104
W_STREAMS = 8
W_ROWS = 144
W_FIRST = 64


def _lane_rounds(lane, rows):
    def cut(a, start, count):
        if start >= rows[a]:
            return [(a, lane, 1, start - rows[a], count)]
        if start + count <= rows[a]:
            return [(a, lane, 0, start, count)]
        return [(a, lane, 0, start, rows[a] - start),
                (a, lane, 1, 0, start + count - rows[a])]

    def block(a, j):
        return cut(a, j * BLK + SHIFT, BLK - SHIFT) + cut(a, (j + 1) * BLK, SHIFT)

    nblk, nq = rows[1] // BLK, rows[0] // QBLK
    assert nblk * BLK == rows[1] == rows[2] and nq * QBLK == rows[0]
    qs = [cut(0, j * QBLK + SHIFT % QBLK, QBLK) for j in range(nq)]
    rounds = []
    for j in range(nblk):
        mine = qs[j * nq // nblk:(j + 1) * nq // nblk]
        if lane % 2 == 0:
            rounds.append([block(1, j)] + mine[:-1] + [block(2, j)] + mine[-1:])
        else:
            rounds.append(mine[:1] + [block(1, j)] + mine[1:] + [block(2, j)])
    return rounds


def _read_schedule(rows):
    lanes = [_lane_rounds(lane, rows) for lane in range(LANES)]
    threads = []
    for t in range(2):
        threads.append([copy + (t,)
                        for step in zip(*lanes[t::2])
                        for visits in step
                        for visit in visits
                        for copy in visit])
    assert len(threads[0]) == len(threads[1])
    return [copy for pair in zip(*threads) for copy in pair]


def _make_kernel(sq, sk, d):
    hl = HB // LANES
    rows = (hl * sq, hl * sk, hl * sk)
    base = (0, rows[0], rows[0] + rows[1])
    sched = _read_schedule(rows)
    nd = len(sched)
    assert all(not copy[2] for copy in sched[:DEPTH])
    scale = (d ** -0.5) * math.log2(math.e)

    def kernel(q_hbm, k_hbm, v_hbm, o_hbm, buf, ob, sem_in, sem_out):
        n = q_hbm.shape[1]
        stream_rows = o_hbm.shape[1]
        stream_chunks = stream_rows // rows[0]
        lane_streams = W_STREAMS // LANES
        assert stream_chunks * lane_streams == n
        hbm = (q_hbm, k_hbm, v_hbm)

        def start_read(copy, chunk, slot):
            a, lane, _, row, count, thread = copy
            pltpu.make_async_copy(
                hbm[a].at[lane, chunk, pl.ds(row, count), :],
                buf.at[slot, lane, pl.ds(base[a] + row, count), :],
                sem_in.at[slot],
            ).start(priority=thread)

        def start_reads(lo, hi, i, slots):
            for t in range(lo, hi):
                copy = sched[t % nd]
                ahead = t // nd + copy[2]
                if ahead in slots:
                    start_read(copy, i + ahead, slots[ahead])

        def wait_reads(slot):
            pltpu.make_async_copy(buf.at[slot], buf.at[slot], sem_in.at[slot]).wait()

        def start_write(w, carry):
            part = pl.ds(pl.multiple_of(w * W_ROWS, 16), W_ROWS)
            pltpu.make_async_copy(
                ob.at[:, part, :], o_hbm.at[:, part, :], sem_out).start()
            return carry

        def attend(i, after_head):
            slot = i % RING
            stream = i // stream_chunks
            out_row = (i % stream_chunks) * rows[0]
            for h in range(HB):
                lane, hh = divmod(h, hl)
                q = buf[slot, lane, pl.ds(base[0] + hh * sq, sq), :]
                k = buf[slot, lane, pl.ds(base[1] + hh * sk, sk), :]
                v = buf[slot, lane, pl.ds(base[2] + hh * sk, sk), :]
                s = lax.dot_general(q, k, (((1,), (1,)), ((), ())),
                                    preferred_element_type=jnp.float32)
                m = jnp.max(s, axis=-1, keepdims=True)
                p = jnp.exp2((s - m) * scale)
                l = jnp.sum(p, axis=-1, keepdims=True)
                o = jnp.dot(p.astype(v.dtype), v, preferred_element_type=jnp.float32)
                r = pl.reciprocal(l, approx=True)
                r = r * (2.0 - l * r)
                ob[lane * lane_streams + stream,
                   pl.ds(pl.multiple_of(out_row + hh * sq, 16), sq), :] = (
                       (o * r).astype(ob.dtype))
                after_head(h)

        lead = nd + DEPTH
        n_main = n - (RING - 1)
        for copy in sched:
            if copy[2]:
                start_read(copy, 0, 0)
        start_reads(0, lead, 0, {0: 0, 1: 1})

        def main_step(i, carry):
            slots = {ahead: (i + ahead) % RING for ahead in (1, 2)}
            wait_reads(i % RING)
            attend(i, lambda h: start_reads(
                lead + (h * nd) // HB, lead + ((h + 1) * nd) // HB, i, slots))
            return carry

        lax.fori_loop(0, n_main, main_step, 0)
        start_reads(DEPTH, nd, n - 1, {0: (n - 1) % RING})

        assert W_FIRST * W_ROWS <= stream_rows - (n - n_main) * rows[0]
        lax.fori_loop(0, W_FIRST, start_write, 0)
        for j in range(n_main, n):
            wait_reads(j % RING)

        def tail_step(i, carry):
            attend(i, lambda h: None)
            return carry

        lax.fori_loop(n_main, n, tail_step, 0)
        lax.fori_loop(W_FIRST, stream_rows // W_ROWS, start_write, 0)
        pltpu.make_async_copy(ob, o_hbm, sem_out).wait()

    return kernel, rows


@jax.jit
def pallas_standalone__mha_softmax__near_ridge_kernel(
    q: jax.Array,
    k: jax.Array,
    v: jax.Array,
):
    b, h, sq, d = q.shape
    sk = k.shape[2]
    n = b * h // HB
    stream_rows = b * h * sq // W_STREAMS
    assert stream_rows % W_ROWS == 0
    kernel, rows = _make_kernel(sq, sk, d)
    out = pl.pallas_call(
        kernel,
        in_specs=[pl.BlockSpec(memory_space=pl.ANY)] * 3,
        out_specs=pl.BlockSpec(memory_space=pl.ANY),
        out_shape=jax.ShapeDtypeStruct((W_STREAMS, stream_rows, d), q.dtype),
        scratch_shapes=[
            pltpu.VMEM((RING, LANES, sum(rows), d), q.dtype),
            pltpu.VMEM((W_STREAMS, stream_rows, d), q.dtype),
            pltpu.SemaphoreType.DMA((RING,)),
            pltpu.SemaphoreType.DMA(()),
        ],
        compiler_params=pltpu.CompilerParams(
            vmem_limit_bytes=104 * 1024 * 1024,
            disable_bounds_checks=True,
        ),
    )(q.reshape(LANES, n, rows[0], d),
      k.reshape(LANES, n, rows[1], d),
      v.reshape(LANES, n, rows[2], d))
    return out.reshape(b, h, sq, d)
```

```python
import math

import jax
import jax.numpy as jnp
from jax import lax
import jax.experimental.pallas as pl
import jax.experimental.pallas.tpu as pltpu

HB = 16
LANES = 4
RING = 3
DEPTH = 70
BLK = 256
QBLK = 128
SHIFT = 104
W_STRIDE = 4096
W_STREAMS = 8
W_ROWS = 64
W_FIRST = 64
W_STEP = 32


def _lane_rounds(lane, rows):
    def cut(a, start, count):
        if start >= rows[a]:
            return [(a, lane, 1, start - rows[a], count)]
        if start + count <= rows[a]:
            return [(a, lane, 0, start, count)]
        return [(a, lane, 0, start, rows[a] - start),
                (a, lane, 1, 0, start + count - rows[a])]

    def block(a, j):
        return cut(a, j * BLK + SHIFT, BLK - SHIFT) + cut(a, (j + 1) * BLK, SHIFT)

    nblk, nq = rows[1] // BLK, rows[0] // QBLK
    assert nblk * BLK == rows[1] == rows[2] and nq * QBLK == rows[0]
    qs = [cut(0, j * QBLK + SHIFT % QBLK, QBLK) for j in range(nq)]
    rounds = []
    for j in range(nblk):
        mine = qs[j * nq // nblk:(j + 1) * nq // nblk]
        if lane % 2 == 0:
            rounds.append([block(1, j)] + mine[:-1] + [block(2, j)] + mine[-1:])
        else:
            rounds.append(mine[:1] + [block(1, j)] + mine[1:] + [block(2, j)])
    return rounds


def _read_schedule(rows):
    lanes = [_lane_rounds(lane, rows) for lane in range(LANES)]
    threads = []
    for t in range(2):
        threads.append([copy + (t,)
                        for step in zip(*lanes[t::2])
                        for visits in step
                        for visit in visits
                        for copy in visit])
    assert len(threads[0]) == len(threads[1])
    return [copy for pair in zip(*threads) for copy in pair]


def _make_kernel(sq, sk, d):
    hl = HB // LANES
    rows = (hl * sq, hl * sk, hl * sk)
    base = (0, rows[0], rows[0] + rows[1])
    sched = _read_schedule(rows)
    nd = len(sched)
    assert all(not copy[2] for copy in sched[:DEPTH])
    scale = (d ** -0.5) * math.log2(math.e)
    piece = math.gcd(sq, W_STRIDE)
    assert piece % 16 == 0

    def kernel(q_hbm, k_hbm, v_hbm, o_hbm, buf, ob, sem_in, sem_out):
        n = q_hbm.shape[1]
        lane_rows = n * rows[0]
        groups = o_hbm.shape[0] // W_STREAMS
        group_rows = W_STREAMS * W_STRIDE
        per_group = W_STRIDE // W_ROWS
        hbm = (q_hbm, k_hbm, v_hbm)

        def start_read(copy, chunk, slot):
            a, lane, _, row, count, thread = copy
            pltpu.make_async_copy(
                hbm[a].at[lane, chunk, pl.ds(row, count), :],
                buf.at[slot, lane, pl.ds(base[a] + row, count), :],
                sem_in.at[slot],
            ).start(priority=thread)

        def start_reads(lo, hi, i, slots):
            for t in range(lo, hi):
                copy = sched[t % nd]
                ahead = t // nd + copy[2]
                if ahead in slots:
                    start_read(copy, i + ahead, slots[ahead])

        def wait_reads(slot):
            pltpu.make_async_copy(buf.at[slot], buf.at[slot], sem_in.at[slot]).wait()

        def attend(i, after_head):
            slot = lax.rem(i, RING)
            for h in range(HB):
                lane, hh = divmod(h, hl)
                q = buf[slot, lane, pl.ds(base[0] + hh * sq, sq), :]
                k = buf[slot, lane, pl.ds(base[1] + hh * sk, sk), :]
                v = buf[slot, lane, pl.ds(base[2] + hh * sk, sk), :]
                s = lax.dot_general(q, k, (((1,), (1,)), ((), ())),
                                    preferred_element_type=jnp.float32)
                m = jnp.max(s, axis=-1, keepdims=True)
                p = jnp.exp2((s - m) * scale)
                l = jnp.sum(p, axis=-1, keepdims=True)
                o = jnp.dot(p.astype(v.dtype), v, preferred_element_type=jnp.float32)
                r = pl.reciprocal(l, approx=True)
                r = r * (2.0 - l * r)
                o = (o * r).astype(ob.dtype)
                for j in range(0, sq, piece):
                    row = i * rows[0] + (lane * lane_rows + hh * sq + j)
                    at = pl.multiple_of(lax.rem(row, W_STRIDE), piece)
                    ob[lax.div(row, W_STRIDE), pl.ds(at, piece), :] = o[j:j + piece]
                after_head(h)

        n_main = n - (RING - 1)
        pending = [(lane * lane_rows + n_main * rows[0], (lane + 1) * lane_rows)
                   for lane in range(LANES)]
        done = [g for g in range(groups)
                if not any(g * group_rows < hi and lo < (g + 1) * group_rows
                           for lo, hi in pending)]
        order = done + [g for g in range(groups) if g not in done]
        early = W_FIRST + (n - n_main) * W_STEP
        assert early <= len(done) * per_group

        def start_write(w, carry):
            j = lax.div(w, per_group)
            g = jnp.int32(order[0])
            for u in range(1, groups):
                g = jnp.where(j >= u, order[u], g)
            streams = pl.ds(g * W_STREAMS, W_STREAMS)
            part = pl.ds(pl.multiple_of(lax.rem(w, per_group) * W_ROWS, 16), W_ROWS)
            pltpu.make_async_copy(
                ob.at[streams, part, :], o_hbm.at[streams, part, :], sem_out).start()
            return carry

        lead = nd + DEPTH
        for copy in sched:
            if copy[2]:
                start_read(copy, 0, 0)
        start_reads(0, lead, 0, {0: 0, 1: 1})

        def main_step(i, carry):
            slots = {ahead: lax.rem(i + ahead, RING) for ahead in (1, 2)}
            wait_reads(lax.rem(i, RING))
            attend(i, lambda h: start_reads(
                lead + (h * nd) // HB, lead + ((h + 1) * nd) // HB, i, slots))
            return carry

        lax.fori_loop(0, n_main, main_step, 0)
        start_reads(DEPTH, nd, n - 1, {0: (n - 1) % RING})
        lax.fori_loop(0, W_FIRST, start_write, 0)
        for j in range(n_main, n):
            wait_reads(j % RING)

        def tail_step(i, carry):
            attend(i, lambda h: None)
            lo = W_FIRST + (i - n_main) * W_STEP
            lax.fori_loop(lo, lo + W_STEP, start_write, 0)
            return carry

        lax.fori_loop(n_main, n, tail_step, 0)
        lax.fori_loop(early, groups * per_group, start_write, 0)
        pltpu.make_async_copy(ob, o_hbm, sem_out).wait()

    return kernel, rows


@jax.jit
def pallas_standalone__mha_softmax__near_ridge_kernel(
    q: jax.Array,
    k: jax.Array,
    v: jax.Array,
):
    b, h, sq, d = q.shape
    sk = k.shape[2]
    n = b * h // HB
    streams = b * h * sq // W_STRIDE
    assert streams * W_STRIDE == b * h * sq and streams % W_STREAMS == 0
    kernel, rows = _make_kernel(sq, sk, d)
    out = pl.pallas_call(
        kernel,
        in_specs=[pl.BlockSpec(memory_space=pl.ANY)] * 3,
        out_specs=pl.BlockSpec(memory_space=pl.ANY),
        out_shape=jax.ShapeDtypeStruct((streams, W_STRIDE, d), q.dtype),
        scratch_shapes=[
            pltpu.VMEM((RING, LANES, sum(rows), d), q.dtype),
            pltpu.VMEM((streams, W_STRIDE, d), q.dtype),
            pltpu.SemaphoreType.DMA((RING,)),
            pltpu.SemaphoreType.DMA(()),
        ],
        compiler_params=pltpu.CompilerParams(
            vmem_limit_bytes=104 * 1024 * 1024,
            disable_bounds_checks=True,
        ),
    )(q.reshape(LANES, n, rows[0], d),
      k.reshape(LANES, n, rows[1], d),
      v.reshape(LANES, n, rows[2], d))
    return out.reshape(b, h, sq, d)
```
